```python
import jax
import jax.numpy as jnp

def _softmax(x, axis=-1):
    return jax.nn.softmax(x, axis=axis)
def _gelu(x):
    return jax.nn.gelu(x, approximate=True)
def _silu(x):
    return jax.nn.silu(x)
def _sigmoid(x):
    return jax.nn.sigmoid(x)
def _layernorm(x, axis=-1, eps=1e-5):
    m = jnp.mean(x, axis=axis, keepdims=True)
    v = jnp.var(x, axis=axis, keepdims=True)
    return (x - m) / jnp.sqrt(v + eps)
def _scatter_add(tgt, idx, src, axis=0):
    return tgt.at[idx].add(src)
def _segment_sum(src, seg, n):
    return jax.ops.segment_sum(src, seg, n)
class _Rng:
    def __init__(self, key):
        self._k = key
    def _next(self):
        self._k, sub = jax.random.split(self._k)
        return sub
    def normal(self, shape):
        return jax.random.normal(self._next(), shape, dtype=jnp.bfloat16)
    def randint(self, lo, hi, shape):
        return jax.random.randint(self._next(), shape, lo, hi, dtype=jnp.int32)
    def uniform(self, shape, lo=0.0, hi=1.0):
        return jax.random.uniform(self._next(), shape, jnp.bfloat16, lo, hi)
    def permutation(self, n):
        return jax.random.permutation(self._next(), n)


kernel_name = 'standalone__batchnorm__sampling'

def setup_inputs():
    _rng = _Rng(jax.random.key(int.from_bytes(__import__("os").urandom(4), "little")))
    _w = (lambda a: (lambda t: t.astype(jnp.bfloat16) if jnp.issubdtype(t.dtype, jnp.floating) else t)(jnp.asarray(a)))
    B, S, C = 1024, 32, 576
    K = 3
    return {
        "x": _w((lambda *s: _rng.normal(s) * 0.05)(B, S, C)),
        "w": _w((lambda *s: _rng.normal(s) * 0.05)(K, C, C) * (1.0 / (K * C) ** 0.5)),
        "mean": _w((lambda *s: _rng.normal(s) * 0.05)(C) * 0.1),
        "var": _w(jnp.abs((lambda *s: _rng.normal(s) * 0.05)(C)) + 0.5),
        "g": _w((lambda *s: _rng.normal(s) * 0.05)(C) + 1.0),
        "b": _w((lambda *s: _rng.normal(s) * 0.05)(C) * 0.1),
    }

def reference(x, w, mean, var, g, b):
    K = 3
    P = K // 2
    S = x.shape[1]
    xp = jnp.pad(x, ((0, 0), (P, P), (0, 0)))
    y = sum(jnp.einsum('bsc,cd->bsd', xp[:, k:k + S, :], w[k]) for k in range(K))
    inv_std = 1.0 / jnp.sqrt(var + 1e-5)
    y = (y - mean) * (g * inv_std) + b
    return _silu(y)
```

```python
import jax
import jax.numpy as jnp
from jax import lax
import jax.experimental.pallas as pl
import jax.experimental.pallas.tpu as pltpu

F32 = jnp.float32
BF16 = jnp.bfloat16


def _prepare_weights(w_ref, mean_ref, var_ref, g_ref, b_ref, u_ref, sh_ref):
    C = w_ref.shape[-1]
    scale = g_ref[...].astype(F32) * (1.0 / jnp.sqrt(var_ref[...].astype(F32) + 1e-5))
    shift = b_ref[...].astype(F32) - mean_ref[...].astype(F32) * scale
    scale = (0.5 * scale).reshape(1, C)
    shift = (0.5 * shift).reshape(1, C)
    sh_ref[...] = jnp.broadcast_to(shift, (128, C)).T
    w0, w1, w2 = [w_ref[k].astype(F32) * scale for k in range(3)]

    def put(t, v):
        u_ref[t] = v.astype(BF16).T

    e = w0 + w2
    put(0, w0 * 0.25)
    put(1, (e + w1) * (-1 / 6))
    put(2, (e - w1) * (-1 / 6))
    p = w0 * (1 / 24) + w2 * (1 / 6)
    q = w1 * (1 / 12)
    put(3, p + q)
    put(4, p - q)
    put(5, w2)


def _silu_half(h):
    return (h * jnp.tanh(h) + h).astype(BF16)


def _kernel(x_ref, w_ref, mean_ref, var_ref, g_ref, b_ref, o_ref, u_ref, sh_ref):
    @pl.when(pl.program_id(0) == 0)
    def _():
        _prepare_weights(w_ref, mean_ref, var_ref, g_ref, b_ref, u_ref, sh_ref)

    def tile(j, first, last):
        ld = lambda i: x_ref[4 * j - 1 + i].astype(F32)
        d1, d2, d3, d4 = ld(1), ld(2), ld(3), ld(4)
        a = d4 - 4.0 * d2
        bb = d3 - 4.0 * d1
        v1 = (a + bb).astype(BF16)
        v2 = (a - bb).astype(BF16)
        c = d4 - d2
        e = 2.0 * (d3 - d1)
        v3 = (c + e).astype(BF16)
        v4 = (c - e).astype(BF16)
        v0 = d4 - 5.0 * d2
        if not first:
            v0 = v0 + 4.0 * ld(0)
        v5 = 4.0 * d1 - 5.0 * d3
        if not last:
            v5 = v5 + ld(5)
        v0 = v0.astype(BF16)
        v5 = v5.astype(BF16)
        dot = lambda t, v: jnp.dot(u_ref[t], v, preferred_element_type=F32)
        m1 = dot(1, v1) + sh_ref[...]
        m2 = dot(2, v2)
        s12 = m1 + m2
        d12 = m1 - m2
        m3 = dot(3, v3)
        m4 = dot(4, v4)
        s34 = m3 + m4
        d34 = m3 - m4
        o_ref[4 * j + 1] = _silu_half(d12 + 2.0 * d34)
        o_ref[4 * j + 2] = _silu_half(s12 + 4.0 * s34)
        o_ref[4 * j] = _silu_half(dot(0, v0) + (s12 + s34))
        o_ref[4 * j + 3] = _silu_half((d12 + 8.0 * d34) + dot(5, v5))

    n = x_ref.shape[0] // 4
    for j in range(n):
        tile(j, j == 0, j == n - 1)


@jax.jit
def pallas_standalone__batchnorm__sampling_kernel(x, w, mean, var, g, b):
    B, S, C = x.shape
    bt = 128
    xt = jnp.transpose(x, (1, 2, 0))
    vec = pl.BlockSpec((C,), lambda i: (0,))
    out = pl.pallas_call(
        _kernel,
        grid=(B // bt,),
        in_specs=[
            pl.BlockSpec((S, C, bt), lambda i: (0, 0, i)),
            pl.BlockSpec((3, C, C), lambda i: (0, 0, 0)),
            vec, vec, vec, vec,
        ],
        out_specs=pl.BlockSpec((S, C, bt), lambda i: (0, 0, i)),
        out_shape=jax.ShapeDtypeStruct((S, C, B), BF16),
        scratch_shapes=[pltpu.VMEM((6, C, C), BF16), pltpu.VMEM((C, 128), F32)],
        compiler_params=pltpu.CompilerParams(
            dimension_semantics=("arbitrary",),
            vmem_limit_bytes=64 * 1024 * 1024,
        ),
    )(xt, w, mean, var, g, b)
    return jnp.transpose(out, (2, 0, 1))
```

```python
import jax
import jax.numpy as jnp
from jax import lax
import jax.experimental.pallas as pl
import jax.experimental.pallas.tpu as pltpu

F32 = jnp.float32
BF16 = jnp.bfloat16
BT = 128
X_CUT = 2
O_CUTS = (6, 7)


def _silu_half(h):
    return (h * jnp.tanh(h) + h).astype(BF16)


def _kernel(x_hbm, w_hbm, mean_ref, var_ref, g_ref, b_ref, o_hbm,
            u_ref, sh_ref, xb, ob, w_ref, xs, osem, ws):
    S, C, B = x_hbm.shape
    nb, nt, nk = B // BT, S // 4, pl.cdiv(C, 128)

    def lanes(i):
        return pl.ds(i * BT if isinstance(i, int) else pl.multiple_of(i * BT, BT), BT)

    def xcopy(i, lo=0, hi=S, c=0):
        return pltpu.make_async_copy(
            x_hbm.at[lo:hi, :, lanes(i)], xb.at[i % 2, lo:hi], xs.at[i % 2, c])

    def ocopy(i, lo=0, hi=S, c=0):
        return pltpu.make_async_copy(
            ob.at[i % 2, lo:hi], o_hbm.at[lo:hi, :, lanes(i)], osem.at[i % 2, c])

    def wcopy(k):
        r = min(128, C - 128 * k)
        return pltpu.make_async_copy(
            w_hbm.at[:, 128 * k:128 * k + r, :], w_ref.at[:, 128 * k:128 * k + r, :], ws.at[k])

    xc = 4 * X_CUT + 1
    for k in range(nk):
        wcopy(k).start()
    xcopy(0, 0, xc, 0).start()

    scale = g_ref[...].astype(F32) * (1.0 / jnp.sqrt(var_ref[...].astype(F32) + 1e-5))
    shift = b_ref[...].astype(F32) - mean_ref[...].astype(F32) * scale
    scale = (0.5 * scale).reshape(1, C)
    shift = (0.5 * shift).reshape(1, C)
    sh_ref[...] = jnp.broadcast_to(shift, (128, C)).T

    for k in range(nk):
        r = min(128, C - 128 * k)
        wcopy(k).wait()
        if k == nk - 1:
            xcopy(0, xc, S, 1).start()
        w0, w1, w2 = [w_ref[q, 128 * k:128 * k + r, :].astype(F32) * scale for q in range(3)]

        def put(t, v):
            u_ref[t, :, 128 * k:128 * k + r] = v.astype(BF16).T

        e = w0 + w2
        put(1, (e + w1) * (-1 / 6))
        put(2, (e - w1) * (-1 / 6))
        p = w0 * (1 / 24) + w2 * (1 / 6)
        q = w1 * (1 / 12)
        put(3, p + q)
        put(4, p - q)
        put(0, w0 * 0.25)
        put(5, w2)

    def tile(sl, j):
        ld = lambda k: xb[sl, 4 * j - 1 + k].astype(F32)
        d1, d2, d3, d4 = ld(1), ld(2), ld(3), ld(4)
        a = d4 - 4.0 * d2
        bb = d3 - 4.0 * d1
        v1 = (a + bb).astype(BF16)
        v2 = (a - bb).astype(BF16)
        c = d4 - d2
        e = 2.0 * (d3 - d1)
        v3 = (c + e).astype(BF16)
        v4 = (c - e).astype(BF16)
        v0 = d4 - 5.0 * d2
        if j > 0:
            v0 = v0 + 4.0 * ld(0)
        v5 = 4.0 * d1 - 5.0 * d3
        if j < nt - 1:
            v5 = v5 + ld(5)
        v0 = v0.astype(BF16)
        v5 = v5.astype(BF16)
        dot = lambda t, v: jnp.dot(u_ref[t], v, preferred_element_type=F32)
        m1 = dot(1, v1) + sh_ref[...]
        m2 = dot(2, v2)
        s12 = m1 + m2
        d12 = m1 - m2
        m3 = dot(3, v3)
        m4 = dot(4, v4)
        s34 = m3 + m4
        d34 = m3 - m4
        ob[sl, 4 * j + 1] = _silu_half(d12 + 2.0 * d34)
        ob[sl, 4 * j + 2] = _silu_half(s12 + 4.0 * s34)
        ob[sl, 4 * j] = _silu_half(dot(0, v0) + (s12 + s34))
        ob[sl, 4 * j + 3] = _silu_half((d12 + 8.0 * d34) + dot(5, v5))

    xcopy(0, 0, xc, 0).wait()
    for j in range(nt):
        if j == X_CUT:
            xcopy(0, xc, S, 1).wait()
            xcopy(1).start()
        tile(0, j)

    def batch(i, carry):
        ocopy(i - 1).start()
        xcopy(i + 1).start()

        @pl.when(i >= 2)
        def _():
            ocopy(i - 2).wait()

        xcopy(i).wait()
        for j in range(nt):
            tile(i % 2, j)
        return carry

    lax.fori_loop(1, nb - 1, batch, 0)

    i = nb - 1
    ocopy(i - 1).start()
    ocopy(i - 2).wait()
    xcopy(i).wait()
    cuts = [0] + [4 * c for c in O_CUTS] + [S]
    for j in range(nt):
        tile(i % 2, j)
        if 4 * (j + 1) in cuts:
            c = cuts.index(4 * (j + 1))
            ocopy(i, cuts[c - 1], cuts[c], c - 1).start()
    ocopy(i - 1).wait()
    for c in range(1, len(cuts)):
        ocopy(i, cuts[c - 1], cuts[c], c - 1).wait()


@jax.jit
def pallas_standalone__batchnorm__sampling_kernel(x, w, mean, var, g, b):
    B, S, C = x.shape
    assert w.shape[0] == 3 and S % 4 == 0 and S // 4 > O_CUTS[-1] and B % BT == 0 and B // BT >= 3
    xt = jnp.transpose(x, (1, 2, 0))
    vec = pl.BlockSpec((C,), lambda i: (0,))
    hbm = pl.BlockSpec(memory_space=pl.ANY)
    out = pl.pallas_call(
        _kernel,
        grid=(1,),
        in_specs=[hbm, hbm, vec, vec, vec, vec],
        out_specs=hbm,
        out_shape=jax.ShapeDtypeStruct((S, C, B), BF16),
        scratch_shapes=[
            pltpu.VMEM((6, C, C), BF16),
            pltpu.VMEM((C, 128), F32),
            pltpu.VMEM((2, S, C, BT), BF16),
            pltpu.VMEM((2, S, C, BT), BF16),
            pltpu.VMEM((3, C, C), BF16),
            pltpu.SemaphoreType.DMA((2, 2)),
            pltpu.SemaphoreType.DMA((2, len(O_CUTS) + 1)),
            pltpu.SemaphoreType.DMA((pl.cdiv(C, 128),)),
        ],
        compiler_params=pltpu.CompilerParams(
            dimension_semantics=("arbitrary",),
            vmem_limit_bytes=64 * 1024 * 1024,
        ),
    )(xt, w, mean, var, g, b)
    return jnp.transpose(out, (2, 0, 1))
```
